```python
import os as _os
_os.environ.setdefault("JAX_PLATFORMS", "cpu")
import jax
import jax.numpy as jnp

def _softmax(x, axis=-1):
    return jax.nn.softmax(x, axis=axis)
def _gelu(x):
    return jax.nn.gelu(x, approximate=True)
def _silu(x):
    return jax.nn.silu(x)
def _sigmoid(x):
    return jax.nn.sigmoid(x)
def _layernorm(x, axis=-1, eps=1e-5):
    m = jnp.mean(x, axis=axis, keepdims=True)
    v = jnp.var(x, axis=axis, keepdims=True)
    return (x - m) / jnp.sqrt(v + eps)
def _scatter_add(tgt, idx, src, axis=0):
    return tgt.at[idx].add(src)
def _segment_sum(src, seg, n):
    return jax.ops.segment_sum(src, seg, n)
class _Rng:
    def __init__(self, key):
        self._k = key
    def _next(self):
        self._k, sub = jax.random.split(self._k)
        return sub
    def normal(self, shape):
        return jax.random.normal(self._next(), shape, dtype=jnp.bfloat16)
    def randint(self, lo, hi, shape):
        return jax.random.randint(self._next(), shape, lo, hi, dtype=jnp.int32)
    def uniform(self, shape, lo=0.0, hi=1.0):
        return jax.random.uniform(self._next(), shape, jnp.bfloat16, lo, hi)
    def permutation(self, n):
        return jax.random.permutation(self._next(), n)


kernel_name = 'concat_heads__sliding_block_cached__compressed_kv_cla__decode'

def setup_inputs():
    _rng = _Rng(jax.random.key(int.from_bytes(__import__("os").urandom(4), "little")))
    _w = (lambda a: (lambda t: t.astype(jnp.bfloat16) if jnp.issubdtype(t.dtype, jnp.floating) else t)(jnp.asarray(a)))
    def _A_setup():
        B, Sq, D = 1, 1, 512
        Hq, Hkv, Sk, Dh = 32, 32, 4096, 128
        assert Hq % Hkv == 0, (Hq, Hkv)
        return {
            "x": _w((lambda *s: _rng.normal(s) * 0.8)(B, Sq, D)),
            "k_cache": _w((lambda *s: _rng.normal(s) * 0.8)(B, Hkv, Sk, Dh)),
            "v_cache": _w((lambda *s: _rng.normal(s) * 0.05)(B, Hkv, Sk, Dh)),
            "wq": _w((lambda *s: _rng.normal(s) * 0.8)(D, Hq * Dh) * (D ** -0.5)),
            "wo": _w((lambda *s: _rng.normal(s) * 0.05)(Hq * Dh, D) * ((Hq * Dh) ** -0.5)),
        }
    _A_in = _A_setup()

    def _B_setup():
        B, H, Sq, Sk, D, M = 1, 32, 1, 4096, 128, 512
        Dc = 4 * D
        return {
            "x": _w((lambda *s: _rng.normal(s) * 1.6)(B, Sq, M)),
            "c_kv": _w((lambda *s: _rng.normal(s) * 0.1)(B, Sk, Dc)),
            "w_q": _w((lambda *s: _rng.normal(s) * 1.6)(M, H, D) * (M ** -0.5)),
            "w_uk": _w((lambda *s: _rng.normal(s) * 1.6)(Dc, H, D) * (Dc ** -0.5)),
            "w_uv": _w((lambda *s: _rng.normal(s) * 0.1)(Dc, H, D) * (Dc ** -0.5)),
            "w_o": _w((lambda *s: _rng.normal(s) * 0.1)(H, D, M) * ((H * D) ** -0.5)),
        }
    _B_in = _B_setup()

    return {
        "A_x": _A_in["x"],
        "A_k_cache": _A_in["k_cache"],
        "A_v_cache": _A_in["v_cache"],
        "A_wq": _A_in["wq"],
        "A_wo": _A_in["wo"],
        "B_x": _B_in["x"],
        "B_c_kv": _B_in["c_kv"],
        "B_w_q": _B_in["w_q"],
        "B_w_uk": _B_in["w_uk"],
        "B_w_uv": _B_in["w_uv"],
        "B_w_o": _B_in["w_o"],
    }

def reference(A_x, A_k_cache, A_v_cache, A_wq, A_wo, B_x, B_c_kv, B_w_q, B_w_uk, B_w_uv, B_w_o):
    def _A_ref(x, k_cache, v_cache, wq, wo):
        B, Sq, D = x.shape
        Hq, Dh = 32, 128
        Hkv, Sk = k_cache.shape[1], k_cache.shape[2]
        W = min(4096, max(256, Sk // 4))
        rep = Hq // Hkv
        q = (lambda x, *d: x.transpose(*d))((x @ wq).reshape(B, Sq, Hq, Dh), 0, 2, 1, 3)
        k = jnp.repeat(k_cache[:, :, Sk - W:, :], rep, axis=1)
        v = jnp.repeat(v_cache[:, :, Sk - W:, :], rep, axis=1)
        scores = jnp.einsum("bhqd,bhkd->bhqk", q, k) * (Dh ** -0.5)
        p = _softmax(scores, axis=-1)
        o = jnp.einsum("bhqk,bhkd->bhqd", p, v)
        return (lambda x, *d: x.transpose(*d))(o, 0, 2, 1, 3).reshape(B, Sq, Hq * Dh) @ wo

    def _B_ref(x, c_kv, w_q, w_uk, w_uv, w_o):
        B, Sq, M = x.shape[0], x.shape[1], x.shape[2]
        Sk = c_kv.shape[1]
        H, D = w_q.shape[1], w_q.shape[2]
        q = jnp.einsum("bqm,mhd->bhqd", x, w_q)
        k = jnp.einsum("bkc,chd->bhkd", c_kv, w_uk)
        v = jnp.einsum("bkc,chd->bhkd", c_kv, w_uv)
        scores = jnp.einsum("bhqd,bhkd->bhqk", q, k) * (D ** -0.5)
        off = Sk - Sq
        qi = jnp.arange(Sq)[:, None]
        kj = jnp.arange(Sk)[None, :]
        cmask = kj <= (qi + off)
        scores = jnp.where(cmask[None, None], scores, -1e9)
        p = _softmax(scores, axis=-1)
        ctx = jnp.einsum("bhqk,bhkd->bhqd", p, v)
        return jnp.einsum("bhqd,hdm->bqm", ctx, w_o)

    a = _A_ref(A_x, A_k_cache, A_v_cache, A_wq, A_wo)
    b = _B_ref(B_x, B_c_kv, B_w_q, B_w_uk, B_w_uv, B_w_o)
    return jnp.concatenate([a, b], axis=-1)
```

```python
import contextlib
import jax
import jax.numpy as jnp
from jax import lax
import jax.experimental.pallas as pl
import jax.experimental.pallas.tpu as pltpu

_BF = jnp.bfloat16
_F32 = jnp.float32
_NN = (((1,), (0,)), ((), ()))
_NT = (((1,), (1,)), ((), ()))

H, D, M, DC, SK, W = 32, 128, 512, 512, 4096, 1024


def _dot(a, b, dn=_NN):
    return lax.dot_general(a, b, dn, preferred_element_type=_F32)


def _iota(shape, d):
    return lax.broadcasted_iota(jnp.int32, shape, d)


def _ds(start, size):
    return pl.ds(start if isinstance(start, int) else pl.multiple_of(start, size), size)


ORDER = (("awq",), ("bwq", "uk"), ("c",), ("k0", "k1"), ("v0", "v1"), ("uv",))


def make(win=32, na=2, skip_compute=False, checks=False, scopes=False, order=ORDER,
         stages=("aq", "q", "qa", "s", "pv", "ex", "as", "sm", "av", "ctx"),
         nt=3, nn=2, npv=3, nex=2):
    phases, ready, s = [], {}, 0
    for units in order:
        phases.append((s, units))
        s += 64 * len(units)
        for u in units:
            ready[u] = s - 1 + win
    assert s == 576
    phases += [(576, ("bwo", "awo")), (688, None), (704, ())]
    nsteps = 704
    bounds = sorted({win} | {ph[0] for ph in phases})

    def kernel(ax_hbm, k_hbm, v_hbm, awq_hbm, awo_hbm, bx_hbm, c_hbm, bwq_hbm, uk_hbm, uv_hbm, bwo_hbm,
               out_ref,
               ax_v, k_v, v_v, awq_v, awo_v, bx_v, c_v, bwq_v, uk_v, uv_v, bwo_v,
               xb_s, z_s, s_s, lat_s, latx_s, q_s, sa_s, l_s, o_s, ctx_s, sems, xsems):
        bufs = dict(bwq=(bwq_hbm, bwq_v), uk=(uk_hbm, uk_v), uv=(uv_hbm, uv_v), c=(c_hbm, c_v),
                    bwo=(bwo_hbm, bwo_v), awo=(awo_hbm, awo_v))

        def views(unit, i, s0, n):
            if unit in ("bwq", "uk", "uv"):
                idx = (pl.ds(s0, n), _ds(i * 64, 64))
            elif unit in ("c", "bwo", "awo"):
                idx = (pl.ds(s0, n), _ds(i * 16, 16))
            elif unit == "awq":
                idx = (pl.ds(s0, n), _ds((i >> 2) * 8, 8), _ds((i & 3) * 1024, 1024))
                return awq_hbm.at[idx], awq_v.at[idx]
            else:
                src, dst = (k_hbm, k_v) if unit[0] == "k" else (v_hbm, v_v)
                h = pl.ds(int(unit[1]) * 16 + (i & 3) * 4 + s0, n)
                r = (i >> 2) * 64
                return src.at[h, _ds(SK - W + r, 64)], dst.at[h, _ds(r, 64)]
            src, dst = bufs[unit]
            return src.at[idx], dst.at[idx]

        def last_round_views(p):
            rows = pl.ds(896 + 32 * (p % 4), 32)
            return (views("bwo", 56 + p // 2, 2 * (p % 2), 2),
                    (awo_hbm.at[p // 4, rows], awo_v.at[p // 4, rows]))

        def retire(step, queues=(0, 1), first=0):
            for q in queues:
                cnt = 2 if first >= 688 else (na, 4 - na)[q]
                d = bwq_v.at[pl.ds(0, cnt), pl.ds(0, 64)]
                pltpu.make_async_copy(d, d, sems.at[q, step & (win - 1)]).wait()

        def tick(s0, t, n, u):
            step = s0 + t * n + u
            if s0 >= win:
                retire(step)
            p0, units = [ph for ph in phases if ph[0] <= s0][-1]
            if units is None:
                pair = last_round_views(step - p0)
            else:
                nu = len(units)
                if isinstance(t, int):
                    unit, i = units[(step - p0) % nu], (step - p0) // nu
                else:
                    assert n % nu == 0
                    unit, i = units[(s0 - p0 + u) % nu], (s0 - p0 + u) // nu + t * (n // nu)
                pair = views(unit, i, 0, na), views(unit, i, na, 4 - na)
            for q, (src, dst) in enumerate(pair):
                pltpu.make_async_copy(src, dst, sems.at[q, step & (win - 1)]).start(priority=q)

        pos = [0]

        def emit(trips, n, body, carry, t0):
            s0 = pos[0]
            pos[0] = s0 + trips * n
            assert pos[0] <= nsteps and not any(s0 < b < pos[0] for b in bounds), (s0, pos[0])

            def step(t, c):
                used = [0]

                def tk(count=1):
                    for _ in range(count):
                        tick(s0, t, n, used[0])
                        used[0] += 1
                if body is not None and not skip_compute:
                    c = body(t + t0, tk, c)
                tk(n - used[0])
                assert used[0] == n
                return c
            nm = f"s{s0:03d}_{trips}x{n}_{body.__name__ if body else 'idle'}"
            with (jax.named_scope(nm) if scopes else contextlib.nullcontext()):
                return step(0, carry) if trips == 1 else lax.fori_loop(0, trips, step, carry)

        def idle_until(s1):
            while pos[0] < s1:
                k = min(b for b in bounds + [s1] if b > pos[0]) - pos[0]
                n = 4 if len([ph for ph in phases if ph[0] <= pos[0]][-1][1] or ()) != 3 else 6
                if k >= 2 * n and pos[0] < 688:
                    emit(k // n, n, None, 0, 0)
                else:
                    emit(1, k, None, 0, 0)

        def run(trips, n, body, carry=0, needs=()):
            idle_until(max([ready[u] for u in needs], default=0))
            t0 = 0
            while t0 < trips:
                nxt = min(b for b in bounds if b > pos[0])
                k = min(trips - t0, (nxt - pos[0]) // n)
                if k == 0:
                    idle_until(nxt)
                    continue
                carry = emit(k, n, body, carry, t0)
                t0 += k
            return carry

        scale = D ** -0.5
        row8 = _iota((8, D), 0)
        idle_until(win)
        d_ax = pltpu.make_async_copy(ax_hbm, ax_v, xsems.at[0])
        d_bx = pltpu.make_async_copy(bx_hbm, bx_v, xsems.at[1])
        d_ax.start()
        d_bx.start()
        idle_until(win + 16)
        d_ax.wait()
        d_bx.wait()

        def xb_body(t, tk, c):
            xrow = bx_v[...].astype(_F32)
            for g in range(M // D):
                tk()
                xb_s[g * D:(g + 1) * D, :] = jnp.broadcast_to(xrow[:, g * D:(g + 1) * D], (D, D)).T
                tk(2)
            return c
        run(1, 12, xb_body)
        val = {}

        def stage_q():
            def q_body(t, tk, acc):
                for part in range(4):
                    tk()
                    wblk = bwq_v.at[t >> 1, _ds(((t & 1) * 4 + part) * 16 * H, 16 * H)]
                    xblk = xb_s.at[_ds((t * 4 + part) * 16, 16)]
                    for u in range(16):
                        acc = acc + wblk[u * H:(u + 1) * H, :].astype(_F32) * xblk[u:u + 1, :]
                return acc
            val["qb"] = run(8, 4, q_body, jnp.zeros((H, D), _F32), ("bwq",)).astype(_BF)

        def stage_qa():
            diag = (_iota((H, D), 1) & (H - 1)) == _iota((H, D), 0)

            def qa_body(t, tk, c):
                for u in range(2):
                    tk()
                    r = _dot(val["qb"], uk_v[t >> 1, _ds(((t & 1) * 2 + u) * 1024, 1024), :], _NT)
                    tk()
                    z = jnp.zeros((8, D), _F32)
                    for j in range(8):
                        d = jnp.sum(jnp.where(diag, r[:, j * D:(j + 1) * D], 0.0), axis=0, keepdims=True)
                        z = jnp.where(row8 == j, d, z)
                    z_s[_ds(t * 16 + u * 8, 8), :] = z
                    tk(nt - 2)
                return c
            run(8, 2 * nt, qa_body, 0, ("uk",))

            def perm_body(t, tk, c):
                tk()
                zt = z_s[...].T.astype(_BF)
                lhs = jnp.concatenate([zt[cl * H:(cl + 1) * H, :] for cl in range(4)], axis=1)
                tk()
                rr = _iota((DC, DC), 0)
                perm = (_iota((DC, DC), 1) == 4 * (rr & 127) + (rr >> 7)).astype(_BF)
                tk()
                return _dot(lhs, perm).astype(_BF)
            val["qa"] = run(1, 6, perm_body, jnp.zeros((H, DC), _BF))

        def stage_s():
            def s_body(t, tk, m):
                for u in range(2):
                    tk()
                    s = _dot(val["qa"], c_v[t >> 1, _ds(((t & 1) * 2 + u) * 256, 256), :], _NT) * scale
                    s_s[t * 2 + u] = s
                    m = jnp.maximum(m, jnp.maximum(s[:, :D], s[:, D:]))
                    tk(nt - 1)
                return m
            m = run(8, 2 * nt, s_body, jnp.full((H, D), -jnp.inf, _F32), ("c",))
            val["m"] = jnp.max(m, axis=1, keepdims=True)

        def stage_pv():
            def pv_body(t, tk, carry):
                l, acc = carry
                for u in range(2):
                    tk()
                    p = jnp.exp(s_s[t * 2 + u] - val["m"])
                    l = l + p[:, :D] + p[:, D:]
                    p = p.astype(_BF)
                    tk()
                    acc = acc + _dot(p, c_v[t >> 1, _ds(((t & 1) * 2 + u) * 256, 256), :])
                    tk(npv - 2)
                return l, acc
            l, lat = run(8, 2 * npv, pv_body, (jnp.zeros((H, D), _F32), jnp.zeros((H, DC), _F32)))
            lat = lat / jnp.sum(l, axis=1, keepdims=True)
            lat32 = pltpu.bitcast(lat.astype(_BF), jnp.uint32)
            for g in range(4):
                lat_s[g] = lat32[:, g * D:(g + 1) * D]

        def stage_ex():
            lane = _iota((H // 2, D), 1)
            r2 = 2 * _iota((H // 2, D), 0)
            hl = lane & (H - 1)
            keep = jnp.where(hl == r2, jnp.uint32(0xFFFF),
                             jnp.where(hl == r2 + 1, jnp.uint32(0xFFFF0000), jnp.uint32(0)))

            def ex_body(t, tk, c):
                tk()
                lg = lat_s[t >> 2]
                base = (lane >> 5) + 32 * (t & 3)
                parts = [jnp.take_along_axis(lg, base + 4 * j, axis=1) & keep for j in range(8)]
                latx_s[t] = pltpu.bitcast(jnp.concatenate(parts, axis=1), _BF)
                return c
            run(16, nex, ex_body)

        def stage_ctx():
            def ctx_body(t, tk, acc):
                for u in range(2):
                    tk()
                    acc = acc + _dot(latx_s[t * 2 + u], uv_v[t >> 1, _ds(((t & 1) * 2 + u) * 1024, 1024), :])
                    tk(nn - 1)
                return acc
            ctx_s[...] = run(8, 2 * nn, ctx_body, jnp.zeros((H, D), _F32), ("uv",))

        def stage_aq():
            x8 = jnp.broadcast_to(ax_v[...].astype(_F32), (8, M)).astype(_BF)

            def aq_body(g, tk, c):
                q = jnp.zeros((8, D), _F32)
                for u in range(4):
                    tk()
                    w = awq_v[:, :, _ds(g * 1024 + u * 256, 256)].reshape(M, 256)
                    r = _dot(x8, w)
                    q = jnp.where(row8 == 2 * u, r[:, :D], q)
                    q = jnp.where(row8 == 2 * u + 1, r[:, D:], q)
                    tk(nn - 1)
                q_s[g] = q
                return c
            run(4, 4 * nn, aq_body, 0, ("awq",))

        def stage_as():
            roww = _iota((8, W), 0)

            def as_body(t, tk, s):
                qg = q_s[t >> 2].astype(_BF)
                for u in range(2):
                    tk()
                    s = jnp.where(roww == (t & 3) * 2 + u, _dot(qg, k_v[t * 2 + u], _NT), s)
                    tk(nt - 1)
                sa_s[t >> 2] = s
                return s
            run(16, 2 * nt, as_body, jnp.zeros((8, W), _F32), ("k0", "k1"))

        def stage_sm():
            def sm_body(g, tk, c):
                tk()
                m = jnp.max(sa_s[g] * scale, axis=1, keepdims=True)
                tk()
                p = jnp.exp(sa_s[g] * scale - m)
                sa_s[g] = p
                l_s[g] = jnp.broadcast_to(jnp.sum(p, axis=1, keepdims=True), (8, D))
                return c
            run(4, 4, sm_body)

        def stage_av():
            def av_body(t, tk, o):
                pg = sa_s[t >> 2].astype(_BF)
                for u in range(2):
                    tk()
                    o = jnp.where(row8 == (t & 3) * 2 + u, _dot(pg, v_v[t * 2 + u]), o)
                    tk(nn - 1)
                o_s[_ds((t >> 2) * 8, 8), :] = o / l_s[t >> 2]
                return o
            run(16, 2 * nn, av_body, jnp.zeros((8, D), _F32), ("v0", "v1"))

        todo = dict(q=stage_q, qa=stage_qa, s=stage_s, pv=stage_pv, ex=stage_ex, ctx=stage_ctx,
                    aq=stage_aq, sm=stage_sm, av=stage_av)
        todo["as"] = stage_as
        for name in stages:
            todo[name]()

        def proj(acc, src, w_ref, r, q0, nq):
            if skip_compute:
                return acc
            lhs = jnp.concatenate(
                [jnp.broadcast_to(src[pl.ds((q0 + k) * 8 + r, 1), :], (8, D)) for k in range(nq)], axis=1)
            w = w_ref[q0:q0 + nq, _ds(r * D, D), :].reshape(nq * D, M)
            return acc + _dot(lhs.astype(_BF), w)

        def round_body(r0):
            def proj_body(t, tk, carry):
                acc_a, acc_b = carry
                for q0 in (0, 2):
                    tk()
                    acc_b = proj(acc_b, ctx_s, bwo_v, r0 + t, q0, 2)
                    tk(nn - 1)
                for q0 in (0, 2):
                    tk()
                    acc_a = proj(acc_a, o_s, awo_v, r0 + t, q0, 2)
                    tk(nn - 1)
                return acc_a, acc_b
            return proj_body

        carry = (jnp.zeros((8, M), _F32), jnp.zeros((8, M), _F32))
        r = 0
        while True:
            start = max(pos[0], 576 + 16 * (r + 1) - 1 + win)
            if start + 4 * nn > nsteps:
                break
            idle_until(start)
            carry = run(1, 4 * nn, round_body(r), carry)
            r += 1
        idle_until(nsteps)
        acc_a, acc_b = carry
        done = nsteps - win
        with (jax.named_scope(f"s704_1x{win}_drain") if scopes else contextlib.nullcontext()):
            while r < 7:
                for st in range(done, 576 + 16 * (r + 1)):
                    retire(st)
                done = max(done, 576 + 16 * (r + 1))
                acc_b = proj(acc_b, ctx_s, bwo_v, r, 0, 4)
                acc_a = proj(acc_a, o_s, awo_v, r, 0, 4)
                r += 1
            for st in range(688, 704):
                retire(st, (0,), 688)
            acc_b = proj(acc_b, ctx_s, bwo_v, 7, 0, 4)
            out_ref[:, M:2 * M] = acc_b[0:1].astype(out_ref.dtype)
            for q in range(4):
                for st in range(688 + 4 * q, 692 + 4 * q):
                    retire(st, (1,), 688)
                acc_a = proj(acc_a, o_s, awo_v, 7, q, 1)
            out_ref[:, 0:M] = acc_a[0:1].astype(out_ref.dtype)

    def fn(A_x, A_k_cache, A_v_cache, A_wq, A_wo, B_x, B_c_kv, B_w_q, B_w_uk, B_w_uv, B_w_o):
        hbm = pl.BlockSpec(memory_space=pltpu.HBM)
        V = pltpu.VMEM
        extra = {} if checks else dict(disable_bounds_checks=True, disable_semaphore_checks=True)
        out = pl.pallas_call(
            kernel,
            in_specs=[hbm] * 11,
            out_specs=pl.BlockSpec(memory_space=pltpu.VMEM),
            out_shape=jax.ShapeDtypeStruct((1, 2 * M), A_x.dtype),
            scratch_shapes=[
                V((1, M), _BF), V((H, W, D), _BF), V((H, W, D), _BF),
                V((4, M // 4, H * D), _BF), V((4, H * D // 4, M), _BF), V((1, M), _BF),
                V((4, SK // 4, DC), _BF), V((4, M * H // 4, D), _BF), V((4, DC * H // 4, D), _BF),
                V((4, DC * H // 4, D), _BF), V((4, H * D // 4, M), _BF),
                V((M, D), _F32), V((D, D), _F32), V((16, H, 256), _F32),
                V((4, H // 2, D), jnp.uint32), V((16, H, 1024), _BF), V((H // 8, 8, D), _F32),
                V((H // 8, 8, W), _F32), V((H // 8, 8, D), _F32),
                V((H, D), _F32), V((H, D), _F32),
                pltpu.SemaphoreType.DMA((2, win)), pltpu.SemaphoreType.DMA((2,)),
            ],
            compiler_params=pltpu.CompilerParams(vmem_limit_bytes=64 * 1024 * 1024, **extra),
        )(A_x.reshape(1, M), A_k_cache.reshape(H, SK, D), A_v_cache.reshape(H, SK, D),
          A_wq.reshape(4, M // 4, H * D), A_wo.reshape(4, H * D // 4, M),
          B_x.reshape(1, M), B_c_kv.reshape(4, SK // 4, DC), B_w_q.reshape(4, M * H // 4, D),
          B_w_uk.reshape(4, DC * H // 4, D), B_w_uv.reshape(4, DC * H // 4, D), B_w_o.reshape(4, H * D // 4, M))
        return out.reshape(1, 1, 2 * M)
    return fn


_impl = make(win=64)


@jax.jit
def pallas_concat_heads__sliding_block_cached__compressed_kv_cla__decode_kernel(
        A_x, A_k_cache, A_v_cache, A_wq, A_wo, B_x, B_c_kv, B_w_q, B_w_uk, B_w_uv, B_w_o):
    return _impl(A_x, A_k_cache, A_v_cache, A_wq, A_wo, B_x, B_c_kv, B_w_q, B_w_uk, B_w_uv, B_w_o)
```

```python
import jax
import jax.numpy as jnp
import numpy as np
from jax import lax
import jax.experimental.pallas as pl
import jax.experimental.pallas.tpu as pltpu

H = 32
D = 128
M = 512
DC = 512
SK = 4096
W = min(4096, max(256, SK // 4))

_BF = jnp.bfloat16
_F32 = jnp.float32
_NN = (((1,), (0,)), ((), ()))
_NT = (((1,), (1,)), ((), ()))

_ORDER = (("b_wq", "b_uk"), ("a_wq", "b_c"), ("k0",), ("k1",), ("v0",), ("v1",), ("b_uv",))
_PROJ = 576
_HALF = 672
_DRAIN = 688
_STEPS = 704
_LEAD = (36, 60)
_RING = 64


def _phases():
    phases, ready, s = [], {}, 0
    for units in _ORDER:
        phases.append((s, s + 64 * len(units), units))
        s += 64 * len(units)
        ready.update({u: s for u in units})
    assert s == _PROJ
    phases += [(_PROJ, _HALF, ("b_wo", "a_wo")), (_HALF, _STEPS, None)]
    return phases, ready


def _dot(a, b, dims=_NN):
    return lax.dot_general(a, b, dims, preferred_element_type=_F32)


def _iota(shape, dim):
    return lax.broadcasted_iota(jnp.int32, shape, dim)


def _ds(start, size):
    return pl.ds(start if isinstance(start, int) else pl.multiple_of(start, size), size)


def _kernel(a_x_hbm, k_hbm, v_hbm, a_wq_hbm, a_wo_hbm,
            b_x_hbm, c_hbm, b_wq_hbm, uk_hbm, uv_hbm, b_wo_hbm,
            out_ref,
            a_x, k_buf, v_buf, a_wq, a_wo, b_x, c_buf, b_wq, uk, uv, b_wo,
            xcol_s, z_s, sb_s, lat_s, latx_s, ctx_s, q_s, sa_s, l_s, o_s, flat_s, ocol_s,
            sem0, sem1, x_sems):
    phases, ready = _phases()
    sems = (sem0, sem1)
    weights = dict(b_wq=(b_wq_hbm, b_wq), b_uk=(uk_hbm, uk), b_uv=(uv_hbm, uv), b_c=(c_hbm, c_buf),
                   a_wq=(a_wq_hbm, a_wq), b_wo=(b_wo_hbm, b_wo), a_wo=(a_wo_hbm, a_wo))

    def pieces(unit, i, first):
        if unit[0] in "kv":
            src, dst = (k_hbm, k_buf) if unit[0] == "k" else (v_hbm, v_buf)
            heads = pl.ds(int(unit[1]) * 16 + (i & 3) * 4 + first, 2)
            row = (i >> 2) * 64
            return src.at[heads, _ds(SK - W + row, 64)], dst.at[heads, _ds(row, 64)]
        if unit == "a_wq":
            idx = (pl.ds(first, 2), _ds((i >> 2) * 8, 8), _ds((i & 3) * 1024, 1024))
        elif unit in ("b_wq", "b_uk", "b_uv"):
            idx = (pl.ds(first, 2), _ds(i * 64, 64))
        else:
            idx = (pl.ds(first, 2), _ds(i * 16, 16))
        src, dst = weights[unit]
        return src.at[idx], dst.at[idx]

    def start(queue, step, lo, hi):
        for p0, p1, units in phases:
            if hi < p0 or lo >= p1:
                continue

            def go(p0=p0, units=units):
                p = step - p0
                if units is None:
                    src, dst = pieces(("b_wo", "a_wo")[queue], 48 + (p >> 4) * 8 + (p & 7), (p >> 2) & 2)
                elif len(units) == 2:
                    src, dst = pieces(units[(lo - p0) % 2], p >> 1, 2 * queue)
                else:
                    src, dst = pieces(units[0], p, 2 * queue)
                pltpu.make_async_copy(src, dst, sems[queue].at[step & (_RING - 1)]).start(priority=queue)

            if p0 <= lo and hi < p1:
                go()
            else:
                pl.when((step >= p0) & (step < p1))(go)

    def finish(queue, step):
        same_size = b_wq.at[pl.ds(0, 2), pl.ds(0, 64)]
        pltpu.make_async_copy(same_size, same_size, sems[queue].at[step & (_RING - 1)]).wait()

    now = [0]

    def run(trips, n, body=None, carry=0, needs=()):
        idle_until(max([ready[u] for u in needs], default=0))
        s0 = now[0]
        now[0] = s0 + trips * n
        assert now[0] <= _DRAIN and (trips == 1 or n % 2 == 0)

        def trip(t, carry):
            used = [0]

            def tick(count=1):
                for _ in range(count):
                    lo = s0 + used[0]
                    hi = lo + (trips - 1) * n
                    step = lo + t * n
                    finish(1, step)
                    finish(0, step)
                    for queue, lead in enumerate(_LEAD):
                        start(queue, step + lead, lo + lead, hi + lead)
                    used[0] += 1

            if body is not None:
                carry = body(t, tick, carry)
            assert used[0] <= n
            tick(n - used[0])
            return carry

        return trip(0, carry) if trips == 1 else lax.fori_loop(0, trips, trip, carry)

    def idle_until(step):
        if step - now[0] >= 8:
            run((step - now[0]) // 4, 4)
        if step > now[0]:
            run(1, step - now[0])

    gap = _LEAD[1] - _LEAD[0]

    def fill_one(t, carry):
        for u in range(2):
            start(1, 2 * t + u, u, gap - 2 + u)
        return carry

    def fill_both(t, carry):
        for u in range(2):
            start(0, 2 * t + u, u, _LEAD[0] - 2 + u)
            start(1, gap + 2 * t + u, gap + u, _LEAD[1] - 2 + u)
        return carry

    lax.fori_loop(0, gap // 2, fill_one, 0)
    lax.fori_loop(0, _LEAD[0] // 2, fill_both, 0)
    x_copies = (pltpu.make_async_copy(a_x_hbm, a_x, x_sems.at[0]),
                pltpu.make_async_copy(b_x_hbm, b_x, x_sems.at[1]))
    for copy in x_copies:
        copy.start()
    idle_until(16)
    for copy in x_copies:
        copy.wait()

    scale = D ** -0.5
    row8 = _iota((8, D), 0)

    def x_column(t, tick, carry):
        xrow = b_x[...].astype(_F32)
        for g in range(M // D):
            tick()
            xcol_s[g * D:(g + 1) * D, :] = jnp.broadcast_to(xrow[:, g * D:(g + 1) * D], (D, D)).T
            tick(2)
        return carry

    run(1, 12, x_column)

    def b_query(t, tick, acc):
        for part in range(4):
            tick()
            w = b_wq.at[t >> 1, _ds(((t & 1) * 4 + part) * 16 * H, 16 * H)]
            x = xcol_s.at[_ds((t * 4 + part) * 16, 16)]
            for u in range(16):
                acc = acc + w[u * H:(u + 1) * H, :].astype(_F32) * x[u:u + 1, :]
        return acc

    qb = run(8, 4, b_query, jnp.zeros((H, D), _F32), ("b_wq",)).astype(_BF)

    own_head = (_iota((H, D), 1) & (H - 1)) == _iota((H, D), 0)

    def b_absorb(t, tick, carry):
        for u in range(2):
            tick()
            r = _dot(qb, uk[t >> 1, _ds(((t & 1) * 2 + u) * 1024, 1024), :], _NT)
            tick()
            z = jnp.zeros((8, D), _F32)
            for j in range(8):
                diag = jnp.sum(jnp.where(own_head, r[:, j * D:(j + 1) * D], 0.0), axis=0, keepdims=True)
                z = jnp.where(row8 == j, diag, z)
            z_s[_ds(t * 16 + u * 8, 8), :] = z
            tick()
        return carry

    run(8, 6, b_absorb, 0, ("b_uk",))

    def b_reorder(t, tick, carry):
        tick()
        zt = z_s[...].T.astype(_BF)
        lhs = jnp.concatenate([zt[j * H:(j + 1) * H, :] for j in range(4)], axis=1)
        tick()
        src = _iota((DC, DC), 0)
        order = (_iota((DC, DC), 1) == 4 * (src & (D - 1)) + (src >> 7)).astype(_BF)
        tick()
        return _dot(lhs, order).astype(_BF)

    q_abs = run(1, 6, b_reorder)

    def latent_rows(t, u):
        return c_buf[t >> 1, _ds(((t & 1) * 2 + u) * 256, 256), :]

    def b_scores(t, tick, top):
        for u in range(2):
            tick()
            s = _dot(q_abs, latent_rows(t, u), _NT) * scale
            sb_s[t * 2 + u] = s
            top = jnp.maximum(top, jnp.maximum(s[:, :D], s[:, D:]))
            tick(2)
        return top

    top = run(8, 6, b_scores, jnp.full((H, D), -jnp.inf, _F32), ("b_c",))
    top = jnp.max(top, axis=1, keepdims=True)

    def b_values(t, tick, carry):
        total, acc = carry
        for u in range(2):
            tick()
            p = jnp.exp(sb_s[t * 2 + u] - top)
            total = total + p[:, :D] + p[:, D:]
            p = p.astype(_BF)
            tick()
            acc = acc + _dot(p, latent_rows(t, u))
            tick()
        return total, acc

    total, lat = run(8, 6, b_values, (jnp.zeros((H, D), _F32), jnp.zeros((H, DC), _F32)))
    lat = lat / jnp.sum(total, axis=1, keepdims=True)
    lat = pltpu.bitcast(lat.astype(_BF), jnp.uint32)
    for g in range(DC // D):
        lat_s[g] = lat[:, g * D:(g + 1) * D]

    lane = _iota((H // 2, D), 1)
    low_head = 2 * _iota((H // 2, D), 0)
    keep = jnp.where((lane & (H - 1)) == low_head, np.uint32(0x0000FFFF),
                     jnp.where((lane & (H - 1)) == low_head + 1, np.uint32(0xFFFF0000), np.uint32(0)))

    def b_spread(t, tick, carry):
        words = lat_s[t >> 1]
        for u in range(2):
            tick()
            first = (lane >> 5) + 32 * ((t & 1) * 2 + u)
            parts = [jnp.take_along_axis(words, first + 4 * j, axis=1) & keep for j in range(8)]
            latx_s[t * 2 + u] = pltpu.bitcast(jnp.concatenate(parts, axis=1), _BF)
        return carry

    run(8, 2, b_spread)

    x8 = jnp.broadcast_to(a_x[...].astype(_F32), (8, M)).astype(_BF)

    def a_query(g, tick, carry):
        q = jnp.zeros((8, D), _F32)
        for u in range(4):
            tick()
            r = _dot(x8, a_wq[:, :, _ds(g * 8 * D + u * 2 * D, 2 * D)].reshape(M, 2 * D))
            q = jnp.where(row8 == 2 * u, r[:, :D], q)
            q = jnp.where(row8 == 2 * u + 1, r[:, D:], q)
            tick()
        q_s[g] = q
        return carry

    run(4, 8, a_query, 0, ("a_wq",))

    row8w = _iota((8, W), 0)

    def a_scores(t, tick, s):
        q = q_s[t >> 2].astype(_BF)
        for u in range(2):
            tick()
            s = jnp.where(row8w == (t & 3) * 2 + u, _dot(q, k_buf[t * 2 + u], _NT), s)
            tick(2)
        sa_s[t >> 2] = s
        return s

    run(16, 6, a_scores, jnp.zeros((8, W), _F32), ("k0", "k1"))

    def a_softmax(g, tick, carry):
        tick()
        top = jnp.max(sa_s[g] * scale, axis=1, keepdims=True)
        tick()
        p = jnp.exp(sa_s[g] * scale - top)
        sa_s[g] = p
        l_s[g] = jnp.broadcast_to(jnp.sum(p, axis=1, keepdims=True), (8, D))
        return carry

    run(4, 4, a_softmax)

    def a_values(t, tick, o):
        p = sa_s[t >> 2].astype(_BF)
        for u in range(2):
            tick()
            o = jnp.where(row8 == (t & 3) * 2 + u, _dot(p, v_buf[t * 2 + u]), o)
            tick()
        o_s[_ds((t >> 2) * 8, 8), :] = o / l_s[t >> 2]
        return o

    run(16, 4, a_values, jnp.zeros((8, D), _F32), ("v0", "v1"))

    def b_context(t, tick, acc):
        for u in range(2):
            tick()
            acc = acc + _dot(latx_s[t * 2 + u], uv[t >> 1, _ds(((t & 1) * 2 + u) * 1024, 1024), :])
            tick()
        return acc

    ctx_s[...] = run(8, 4, b_context, jnp.zeros((H, D), _F32), ("b_uv",))

    def flatten(r, tick, carry):
        tick()
        for branch, src in enumerate((ctx_s, o_s)):
            rows = [jnp.broadcast_to(src[pl.ds(8 * q + r, 1), :], (8, D)) for q in range(4)]
            flat_s[branch, r] = jnp.concatenate(rows, axis=1).astype(_BF)
        return carry

    run(8, 2, flatten)

    def o_column(q, tick, carry):
        tick()
        o = o_s[pl.ds(8 * q + 7, 1), :].astype(_BF).astype(_F32)
        ocol_s[q] = jnp.broadcast_to(o, (D, D)).T
        return carry

    run(4, 2, o_column)

    def project(acc, branch, r, q0, nq):
        w = (b_wo, a_wo)[branch][pl.ds(q0, nq), _ds(r * D, D), :].reshape(nq * D, M)
        return acc + _dot(flat_s[branch, r, :, pl.ds(q0 * D, nq * D)], w)

    def rounds_from(r0):
        def body(t, tick, acc):
            acc = list(acc)
            for branch in range(2):
                for q0 in (0, 2):
                    tick()
                    acc[branch] = project(acc[branch], branch, r0 + t, q0, 2)
                    tick()
            return tuple(acc)
        return body

    acc = (jnp.zeros((8, M), _F32), jnp.zeros((8, M), _F32))
    r = 0
    while r < 6:
        idle_until(_PROJ + 16 * (r + 1))
        landed = min(6, (now[0] - _PROJ) // 16)
        acc = run(landed - r, 8, rounds_from(r), acc)
        r = landed
    idle_until(_HALF + 8)
    acc_b, acc_a = run(1, 8, lambda t, tick, acc: tuple(project(acc[i], i, 6, 0, 2) for i in range(2)), acc)
    assert now[0] == _DRAIN and min(_LEAD) >= _STEPS - _DRAIN

    acc_b = project(acc_b, 0, 6, 2, 2)
    acc_a = project(acc_a, 1, 6, 2, 2)
    part = jnp.where(_iota((8, M), 0) == 0, acc_a, 0.0)
    p = 0
    for count in (2, 2, 2, 2, 2, 2, 1, 1, 1, 1):
        if p == 6:
            for step in range(_DRAIN, _STEPS):
                finish(0, step)
            acc_b = project(acc_b, 0, 7, 0, 4)
        for step in range(_DRAIN + p, _DRAIN + p + count):
            finish(1, step)
        r0, n = 16 * (p & 7), 16 * count
        for q in (2 * (p >> 3), 2 * (p >> 3) + 1):
            w = a_wo[q, 7 * D + r0:7 * D + r0 + n, :].astype(_F32)
            prod = w * jnp.concatenate([ocol_s[q, r0:r0 + n, :]] * (M // D), axis=1)
            rows = [prod[8 * j:8 * j + 8] for j in range(n // 8)]
            while len(rows) > 1:
                rows = [rows[j] + rows[j + 1] for j in range(0, len(rows), 2)]
            part = part + rows[0]
        p += count
    assert _DRAIN + p == _STEPS
    out = jnp.concatenate([jnp.sum(part, axis=0, keepdims=True), acc_b[0:1]], axis=1)
    out_ref[...] = out.astype(out_ref.dtype)


@jax.jit
def pallas_concat_heads__sliding_block_cached__compressed_kv_cla__decode_kernel(
        A_x, A_k_cache, A_v_cache, A_wq, A_wo, B_x, B_c_kv, B_w_q, B_w_uk, B_w_uv, B_w_o):
    assert A_k_cache.shape == A_v_cache.shape == (1, H, SK, D) and B_c_kv.shape == (1, SK, DC)
    assert B_w_q.shape == (M, H, D) and B_w_uk.shape == B_w_uv.shape == (DC, H, D)
    operands = (
        A_x.reshape(1, M), A_k_cache.reshape(H, SK, D), A_v_cache.reshape(H, SK, D),
        A_wq.reshape(4, M // 4, H * D), A_wo.reshape(4, H * D // 4, M),
        B_x.reshape(1, M), B_c_kv.reshape(4, SK // 4, DC), B_w_q.reshape(4, M * H // 4, D),
        B_w_uk.reshape(4, DC * H // 4, D), B_w_uv.reshape(4, DC * H // 4, D),
        B_w_o.reshape(4, H * D // 4, M))
    buffers = [pltpu.VMEM((H, W, D) if i in (1, 2) else x.shape, _BF) for i, x in enumerate(operands)]
    out = pl.pallas_call(
        _kernel,
        in_specs=[pl.BlockSpec(memory_space=pltpu.HBM)] * len(operands),
        out_specs=pl.BlockSpec(memory_space=pltpu.VMEM),
        out_shape=jax.ShapeDtypeStruct((1, 2 * M), A_x.dtype),
        scratch_shapes=buffers + [
            pltpu.VMEM((M, D), _F32),
            pltpu.VMEM((D, D), _F32),
            pltpu.VMEM((SK // 256, H, 256), _F32),
            pltpu.VMEM((DC // D, H // 2, D), jnp.uint32),
            pltpu.VMEM((DC * H // 1024, H, 1024), _BF),
            pltpu.VMEM((H, D), _F32),
            pltpu.VMEM((H // 8, 8, D), _F32),
            pltpu.VMEM((H // 8, 8, W), _F32),
            pltpu.VMEM((H // 8, 8, D), _F32),
            pltpu.VMEM((H, D), _F32),
            pltpu.VMEM((2, 8, 8, 4 * D), _BF),
            pltpu.VMEM((4, D, D), _F32),
            pltpu.SemaphoreType.DMA((_RING,)),
            pltpu.SemaphoreType.DMA((_RING,)),
            pltpu.SemaphoreType.DMA((2,)),
        ],
        compiler_params=pltpu.CompilerParams(
            vmem_limit_bytes=64 * 1024 * 1024,
            disable_bounds_checks=True,
            disable_semaphore_checks=True),
    )(*operands)
    return out.reshape(1, 1, 2 * M)
```

```python
import jax
import jax.numpy as jnp
import numpy as np
from jax import lax
import jax.experimental.pallas as pl
import jax.experimental.pallas.tpu as pltpu

H = 32
D = 128
M = 512
DC = 512
SK = 4096
W = min(4096, max(256, SK // 4))

_BF = jnp.bfloat16
_F32 = jnp.float32
_NN = (((1,), (0,)), ((), ()))
_NT = (((1,), (1,)), ((), ()))

_ORDER = (("b_wq", "b_uk"), ("b_c", "b_uv"), ("a_wq", "k0"), ("k1",), ("v0",), ("v1",))
_PROJ = 576
_HALF = 672
_STEPS = 704
_SPLIT = (((0, 1),), ((1, 1), (2, 2)))
_LEAD = (20, 33)
_LATE = 10
_GROUPS = (4, 2, 1, 1)
_RING = 64


def _phases():
    phases, ready, s = [], {}, 0
    for units in _ORDER:
        phases.append((s, s + 64 * len(units), units))
        s += 64 * len(units)
        ready.update({u: s for u in units})
    assert s == _PROJ
    phases += [(_PROJ, _HALF, ("b_wo", "a_wo")), (_HALF, _STEPS, None)]
    return phases, ready


def _dot(a, b, dims=_NN):
    return lax.dot_general(a, b, dims, preferred_element_type=_F32)


def _iota(shape, dim):
    return lax.broadcasted_iota(jnp.int32, shape, dim)


def _ds(start, size):
    return pl.ds(start if isinstance(start, int) else pl.multiple_of(start, size), size)


def _kernel(a_x_hbm, k_hbm, v_hbm, a_wq_hbm, a_wo_hbm,
            b_x_hbm, c_hbm, b_wq_hbm, uk_hbm, uv_hbm, b_wo_hbm,
            out_ref,
            a_x, k_buf, v_buf, a_wq, a_wo, b_x, c_buf, b_wq, uk, uv, b_wo,
            xcol_s, z_s, sb_s, latx_s, ctx_s, q_s, sa_s, pa_s, l_s, o_s, flat_s, ocol_s,
            sem0, sem1, x_sems):
    phases, ready = _phases()
    sems = (sem0, sem1)
    weights = dict(b_wq=(b_wq_hbm, b_wq), b_uk=(uk_hbm, uk), b_uv=(uv_hbm, uv), b_c=(c_hbm, c_buf),
                   a_wq=(a_wq_hbm, a_wq), b_wo=(b_wo_hbm, b_wo), a_wo=(a_wo_hbm, a_wo))

    def pieces(unit, i, first, n):
        if unit[0] in "kv":
            src, dst = (k_hbm, k_buf) if unit[0] == "k" else (v_hbm, v_buf)
            heads = pl.ds(int(unit[1]) * 16 + (i & 3) * 4 + first, n)
            row = (i >> 2) * 64
            return src.at[heads, _ds(SK - W + row, 64)], dst.at[heads, _ds(row, 64)]
        if unit == "a_wq":
            idx = (pl.ds(first, n), _ds((i >> 2) * 8, 8), _ds((i & 3) * 1024, 1024))
        elif unit in ("b_wq", "b_uk", "b_uv"):
            idx = (pl.ds(first, n), _ds(i * 64, 64))
        else:
            idx = (pl.ds(first, n), _ds(i * 16, 16))
        src, dst = weights[unit]
        return src.at[idx], dst.at[idx]

    def start(queue, step, lo, hi, first=0, end=_STEPS):
        for p0, p1, units in phases:
            s0, s1 = max(p0, first), min(p1, end)
            if hi < s0 or lo >= s1 or s0 >= s1:
                continue

            def go(p0=p0, units=units):
                p = step - p0
                for first, n in _SPLIT[queue]:
                    if units is None:
                        src, dst = pieces(("b_wo", "a_wo")[first >> 1], 48 + (p >> 4) * 8 + (p & 7),
                                          ((p >> 2) & 2) + (first & 1), n)
                    elif len(units) == 2:
                        src, dst = pieces(units[(lo - p0) % 2], p >> 1, first, n)
                    else:
                        src, dst = pieces(units[0], p, first, n)
                    pltpu.make_async_copy(src, dst, sems[queue].at[step & (_RING - 1)]).start(priority=queue)

            if s0 <= lo and hi < s1:
                go()
            else:
                pl.when((step >= s0) & (step < s1))(go)

    def finish(queue, step):
        same_size = b_wq.at[pl.ds(0, sum(n for _, n in _SPLIT[queue])), pl.ds(0, 64)]
        pltpu.make_async_copy(same_size, same_size, sems[queue].at[step & (_RING - 1)]).wait()

    gap = _LEAD[1] - _LEAD[0]

    def refill(step, lo, hi):
        start(0, step + _LEAD[0], lo + _LEAD[0], hi + _LEAD[0], end=_STEPS - gap)
        start(1, step + _LEAD[1], lo + _LEAD[1], hi + _LEAD[1])
        start(0, step + _LATE, lo + _LATE, hi + _LATE, first=_STEPS - gap)

    now = [0]

    def run(trips, n, body=None, carry=0, needs=()):
        idle_until(max([ready[u] for u in needs], default=0))
        s0 = now[0]
        now[0] = s0 + trips * n
        assert trips == 1 or n % 2 == 0 or not any(
            units and len(units) == 2 and s0 + _LATE < p1 and now[0] + max(_LEAD) > p0
            for p0, p1, units in phases)

        def trip(t, carry):
            used = [0]

            def tick(count=1):
                for _ in range(count):
                    lo = s0 + used[0]
                    hi = lo + (trips - 1) * n
                    step = lo + t * n
                    finish(1, step)
                    finish(0, step)
                    refill(step, lo, hi)
                    used[0] += 1

            if body is not None:
                carry = body(t, tick, carry)
            assert used[0] <= n
            tick(n - used[0])
            return carry

        return trip(0, carry) if trips == 1 else lax.fori_loop(0, trips, trip, carry)

    def idle_until(step):
        if step - now[0] >= 8:
            run((step - now[0]) // 4, 4)
        if step > now[0]:
            run(1, step - now[0])

    def fill_one(t, carry):
        for u in range(2):
            start(1, 2 * t + u, u, gap - 2 + u)
        return carry

    def fill_both(t, carry):
        for u in range(2):
            start(0, 2 * t + u, u, _LEAD[0] - 2 + u)
            start(1, gap + 2 * t + u, gap + u, _LEAD[1] - 2 + u)
        return carry

    lax.fori_loop(0, gap // 2, fill_one, 0)
    if gap % 2:
        start(1, gap - 1, gap - 1, gap - 1)
    assert _LEAD[0] % 2 == 0
    lax.fori_loop(0, _LEAD[0] // 2, fill_both, 0)
    x_copies = (pltpu.make_async_copy(a_x_hbm, a_x, x_sems.at[0]),
                pltpu.make_async_copy(b_x_hbm, b_x, x_sems.at[1]))
    for copy in x_copies:
        copy.start()
    idle_until(16)
    for copy in x_copies:
        copy.wait()

    scale = D ** -0.5
    row8 = _iota((8, D), 0)

    def x_column(t, tick, carry):
        xrow = b_x[...].astype(_F32)
        for g in range(M // D):
            tick()
            xcol_s[g * D:(g + 1) * D, :] = jnp.broadcast_to(xrow[:, g * D:(g + 1) * D], (D, D)).T
            tick(2)
        return carry

    run(1, 12, x_column)

    def b_query(t, tick, acc):
        for part in range(4):
            tick()
            w = b_wq.at[t >> 1, _ds(((t & 1) * 4 + part) * 16 * H, 16 * H)]
            x = xcol_s.at[_ds((t * 4 + part) * 16, 16)]
            for u in range(16):
                acc = acc + w[u * H:(u + 1) * H, :].astype(_F32) * x[u:u + 1, :]
        return acc

    qb = run(8, 4, b_query, jnp.zeros((H, D), _F32), ("b_wq",)).astype(_BF)

    own_head = (_iota((H, D), 1) & (H - 1)) == _iota((H, D), 0)

    def b_absorb(t, tick, carry):
        for u in range(4):
            tick()
            r = _dot(qb, uk[t, u * 1024:(u + 1) * 1024, :], _NT)
            tick()
            z = jnp.zeros((8, D), _F32)
            for j in range(8):
                diag = jnp.sum(jnp.where(own_head, r[:, j * D:(j + 1) * D], 0.0), axis=0, keepdims=True)
                z = jnp.where(row8 == j, diag, z)
            z_s[_ds(t * 32 + u * 8, 8), :] = z
            tick(1 + u % 2)
        return carry

    run(4, 14, b_absorb, 0, ("b_uk",))

    def b_reorder(t, tick, carry):
        tick()
        zt = z_s[...].T.astype(_BF)
        lhs = jnp.concatenate([zt[j * H:(j + 1) * H, :] for j in range(4)], axis=1)
        tick()
        src = _iota((DC, DC), 0)
        order = (_iota((DC, DC), 1) == 4 * (src & (D - 1)) + (src >> 7)).astype(_BF)
        tick()
        return _dot(lhs, order).astype(_BF)

    q_abs = run(1, 6, b_reorder)

    def b_scores(t, tick, top):
        for u in range(4):
            tick()
            s = _dot(q_abs, c_buf[t, u * 256:(u + 1) * 256, :], _NT)
            tick()
            s = s * scale
            sb_s[t * 4 + u] = s
            top = jnp.maximum(top, jnp.maximum(s[:, :D], s[:, D:]))
            tick(1 + u % 2)
        return top

    top = run(4, 14, b_scores, jnp.full((H, D), -jnp.inf, _F32), ("b_c",))
    top = jnp.max(top, axis=1, keepdims=True)

    def b_values(t, tick, carry):
        total, acc = carry
        for u in range(2):
            tick()
            p = jnp.exp(sb_s[t * 2 + u] - top)
            total = total + p[:, :D] + p[:, D:]
            p = p.astype(_BF)
            tick()
            acc = acc + _dot(p, c_buf[t >> 1, _ds(((t & 1) * 2 + u) * 256, 256), :])
            tick()
        return total, acc

    total, lat = run(8, 6, b_values, (jnp.zeros((H, D), _F32), jnp.zeros((H, DC), _F32)))
    lat = lat / jnp.sum(total, axis=1, keepdims=True)
    lat = pltpu.bitcast(lat.astype(_BF), jnp.uint32)
    lat = jnp.concatenate([lat[:, g * D:(g + 1) * D] for g in range(DC // D)], axis=0)

    lane = _iota(lat.shape, 1)
    low_head = 2 * (_iota(lat.shape, 0) & (H // 2 - 1))
    keep = jnp.where((lane & (H - 1)) == low_head, np.uint32(0x0000FFFF),
                     jnp.where((lane & (H - 1)) == low_head + 1, np.uint32(0xFFFF0000), np.uint32(0)))

    def b_spread(t, tick, carry):
        for j in range(8):
            if j % 2 == 0:
                tick()
            words = jnp.take_along_axis(lat, (lane >> 5) + 32 * t + 4 * j, axis=1) & keep
            for g in range(DC // D):
                part = words[g * (H // 2):(g + 1) * (H // 2), :]
                latx_s[g * 4 + t, :, j * D:(j + 1) * D] = pltpu.bitcast(part, _BF)
        return carry

    run(4, 4, b_spread)

    def b_context(t, tick, acc):
        for u in range(4):
            tick()
            acc = acc + _dot(latx_s[t * 4 + u], uv[t, u * 1024:(u + 1) * 1024, :])
            tick(1 + u % 2)
        return acc

    ctx_s[...] = run(4, 10, b_context, jnp.zeros((H, D), _F32), ("b_uv",))

    x8 = jnp.broadcast_to(a_x[...].astype(_F32), (8, M)).astype(_BF)

    def a_query(g, tick, carry):
        q = jnp.zeros((8, D), _F32)
        for u in range(4):
            tick()
            r = _dot(x8, a_wq[:, :, _ds(g * 8 * D + u * 2 * D, 2 * D)].reshape(M, 2 * D))
            q = jnp.where(row8 == 2 * u, r[:, :D], q)
            q = jnp.where(row8 == 2 * u + 1, r[:, D:], q)
            tick()
        q_s[g] = q
        return carry

    run(4, 8, a_query, 0, ("a_wq",))

    row8w = _iota((8, W), 0)

    def a_scores(t, tick, s):
        q = q_s[t >> 1].astype(_BF)
        for u in range(4):
            tick()
            s = jnp.where(row8w == (t & 1) * 4 + u, _dot(q, k_buf[t * 4 + u], _NT), s)
            tick(2)
        sa_s[t >> 1] = s
        return s

    run(8, 12, a_scores, jnp.zeros((8, W), _F32), ("k0", "k1"))

    def a_softmax(t, tick, carry):
        for g in (2 * t, 2 * t + 1):
            tick()
            top = jnp.max(sa_s[g] * scale, axis=1, keepdims=True)
            tick()
            p = jnp.exp(sa_s[g] * scale - top)
            pa_s[g] = p.astype(_BF)
            l_s[_ds(g * 8, 8), :] = jnp.broadcast_to(jnp.sum(p, axis=1, keepdims=True), (8, D))
            tick()
        return carry

    run(2, 6, a_softmax)

    def a_values(g, tick, carry):
        o = jnp.zeros((8, D), _F32)
        for u in range(8):
            tick()
            o = jnp.where(row8 == u, _dot(pa_s[g], v_buf[g * 8 + u]), o)
            tick()
        o_s[_ds(g * 8, 8), :] = o
        return carry

    run(2, 16, a_values, 0, ("v0",))
    run(2, 16, lambda g, tick, carry: a_values(g + 2, tick, carry), 0, ("v1",))
    o_s[...] = o_s[...] / l_s[...]

    def flatten(t, tick, carry):
        for r in (2 * t, 2 * t + 1):
            tick()
            for branch, src in enumerate((ctx_s, o_s)):
                rows = [jnp.broadcast_to(src[pl.ds(8 * q + r, 1), :], (8, D)) for q in range(4)]
                flat_s[branch, r] = jnp.concatenate(rows, axis=1).astype(_BF)
        return carry

    run(4, 2, flatten)

    def column(t, tick, carry):
        for branch, src in enumerate((ctx_s, o_s)):
            tick()
            row = src[pl.ds(8 * (2 + t) + 7, 1), :].astype(_BF).astype(_F32)
            ocol_s[branch, t] = jnp.broadcast_to(row, (D, D)).T
            tick(2)
        return carry

    run(2, 6, column)

    def project(acc, branch, r, q0, nq):
        w = (b_wo, a_wo)[branch][pl.ds(q0, nq), _ds(r * D, D), :].reshape(nq * D, M)
        return acc + _dot(flat_s[branch, r, :, _ds(q0 * D, nq * D)], w)

    def rounds_from(r0):
        def body(t, tick, acc):
            acc = list(acc)
            for branch in range(2):
                tick()
                acc[branch] = project(acc[branch], branch, r0 + t, 0, 4)
                tick(2)
            return tuple(acc)
        return body

    acc = (jnp.zeros((8, M), _F32), jnp.zeros((8, M), _F32))
    r = 0
    while r < 6:
        idle_until(_PROJ + 16 * (r + 1))
        landed = min(6, (now[0] - _PROJ) // 16)
        acc = run(landed - r, 6, rounds_from(r), acc)
        r = landed
    idle_until(_HALF + 8)

    def halves(t, tick, acc):
        return tuple(project(acc[i], i, 6 + (t >> 1), 2 * (t & 1), 2) for i in range(2))

    acc = run(2, 8, halves, acc)
    acc = halves(2, None, acc)

    part = [jnp.where(_iota((8, M), 0) == 0, x, 0.0) for x in acc]
    last, p = now[0], 0
    assert last == _STEPS - 8
    for count in _GROUPS:
        r0, n = 16 * p, 16 * count
        for step in range(last + p, last + p + count):
            finish(0, step)
            finish(1, step)
            refill(step, step, step)
        for branch, w_ref in enumerate((b_wo, a_wo)):
            for q in range(2):
                w = w_ref[2 + q, 7 * D + r0:7 * D + r0 + n, :].astype(_F32)
                prod = w * jnp.concatenate([ocol_s[branch, q, r0:r0 + n, :]] * (M // D), axis=1)
                rows = [prod[8 * j:8 * j + 8] for j in range(n // 8)]
                while len(rows) > 1:
                    rows = [rows[j] + rows[j + 1] for j in range(0, len(rows), 2)]
                part[branch] = part[branch] + rows[0]
        p += count
    assert last + p == _STEPS
    out = jnp.concatenate([jnp.sum(x, axis=0, keepdims=True) for x in part[::-1]], axis=1)
    out_ref[...] = out.astype(out_ref.dtype)


@jax.jit
def pallas_concat_heads__sliding_block_cached__compressed_kv_cla__decode_kernel(
        A_x, A_k_cache, A_v_cache, A_wq, A_wo, B_x, B_c_kv, B_w_q, B_w_uk, B_w_uv, B_w_o):
    assert A_k_cache.shape == A_v_cache.shape == (1, H, SK, D) and B_c_kv.shape == (1, SK, DC)
    assert B_w_q.shape == (M, H, D) and B_w_uk.shape == B_w_uv.shape == (DC, H, D)
    operands = (
        A_x.reshape(1, M), A_k_cache.reshape(H, SK, D), A_v_cache.reshape(H, SK, D),
        A_wq.reshape(4, M // 4, H * D), A_wo.reshape(4, H * D // 4, M),
        B_x.reshape(1, M), B_c_kv.reshape(4, SK // 4, DC), B_w_q.reshape(4, M * H // 4, D),
        B_w_uk.reshape(4, DC * H // 4, D), B_w_uv.reshape(4, DC * H // 4, D),
        B_w_o.reshape(4, H * D // 4, M))
    buffers = [pltpu.VMEM((H, W, D) if i in (1, 2) else x.shape, _BF) for i, x in enumerate(operands)]
    out = pl.pallas_call(
        _kernel,
        in_specs=[pl.BlockSpec(memory_space=pltpu.HBM)] * len(operands),
        out_specs=pl.BlockSpec(memory_space=pltpu.VMEM),
        out_shape=jax.ShapeDtypeStruct((1, 2 * M), A_x.dtype),
        scratch_shapes=buffers + [
            pltpu.VMEM((M, D), _F32),
            pltpu.VMEM((D, D), _F32),
            pltpu.VMEM((SK // 256, H, 256), _F32),
            pltpu.VMEM((DC * H // 1024, H, 1024), _BF),
            pltpu.VMEM((H, D), _F32),
            pltpu.VMEM((H // 8, 8, D), _F32),
            pltpu.VMEM((H // 8, 8, W), _F32),
            pltpu.VMEM((H // 8, 8, W), _BF),
            pltpu.VMEM((H, D), _F32),
            pltpu.VMEM((H, D), _F32),
            pltpu.VMEM((2, 8, 8, 4 * D), _BF),
            pltpu.VMEM((2, 2, D, D), _F32),
            pltpu.SemaphoreType.DMA((_RING,)),
            pltpu.SemaphoreType.DMA((_RING,)),
            pltpu.SemaphoreType.DMA((2,)),
        ],
        compiler_params=pltpu.CompilerParams(
            vmem_limit_bytes=64 * 1024 * 1024,
            disable_bounds_checks=True,
            disable_semaphore_checks=True),
    )(*operands)
    return out.reshape(1, 1, 2 * M)
```

```python
import jax
import jax.numpy as jnp
import numpy as np
from jax import lax
import jax.experimental.pallas as pl
import jax.experimental.pallas.tpu as pltpu

H = 32
D = 128
M = 512
DC = 512
SK = 4096
W = min(4096, max(256, SK // 4))

_BF = jnp.bfloat16
_F32 = jnp.float32
_NN = (((1,), (0,)), ((), ()))
_NT = (((1,), (1,)), ((), ()))

_ORDER = (("b_c", "b_wq", "b_uk", "b_uv"), ("k0", "a_wq"), ("k1",), ("v0",), ("v1",))
_PROJ = 576
_HALF = 688
_STEPS = 704
_LEAD = (30, 56)
_LATE = 12
_GROUPS = (4, 2, 1, 1)
_RING = 64


def _phases():
    phases, ready, s = [], {}, 0
    for units in _ORDER:
        phases.append((s, s + 64 * len(units), units))
        s += 64 * len(units)
        ready.update({u: s for u in units})
    assert s == _PROJ
    phases += [(_PROJ, _HALF, ("b_wo", "a_wo")), (_HALF, _STEPS, None)]
    return phases, ready


def _dot(a, b, dims=_NN):
    return lax.dot_general(a, b, dims, preferred_element_type=_F32)


def _iota(shape, dim):
    return lax.broadcasted_iota(jnp.int32, shape, dim)


def _ds(start, size):
    return pl.ds(start if isinstance(start, int) else pl.multiple_of(start, size), size)


def _kernel(a_x_hbm, k_hbm, v_hbm, a_wq_hbm, a_wo_hbm,
            b_x_hbm, c_hbm, b_wq_hbm, uk_hbm, uv_hbm, b_wo_hbm,
            out_ref,
            a_x, k_buf, v_buf, a_wq, a_wo, b_x, c_buf, b_wq, uk, uv, b_wo,
            xcol_s, z_s, sb_s, latx_s, ctx_s, q_s, sa_s, pa_s, l_s, o_s, flat_s, ocol_s,
            sem0, sem1, x_sems):
    phases, ready = _phases()
    sems = (sem0, sem1)
    weights = dict(b_wq=(b_wq_hbm, b_wq), b_uk=(uk_hbm, uk), b_uv=(uv_hbm, uv), b_c=(c_hbm, c_buf),
                   a_wq=(a_wq_hbm, a_wq), b_wo=(b_wo_hbm, b_wo), a_wo=(a_wo_hbm, a_wo))

    def pieces(unit, i, first):
        if unit[0] in "kv":
            src, dst = (k_hbm, k_buf) if unit[0] == "k" else (v_hbm, v_buf)
            heads = pl.ds(int(unit[1]) * 16 + (i & 3) * 4 + first, 2)
            row = (i >> 2) * 64
            return src.at[heads, _ds(SK - W + row, 64)], dst.at[heads, _ds(row, 64)]
        if unit == "a_wq":
            idx = (pl.ds(first, 2), _ds((i >> 2) * 8, 8), _ds((i & 3) * 1024, 1024))
        elif unit in ("b_wq", "b_uk", "b_uv"):
            idx = (pl.ds(first, 2), _ds(i * 64, 64))
        else:
            idx = (pl.ds(first, 2), _ds(i * 16, 16))
        src, dst = weights[unit]
        return src.at[idx], dst.at[idx]

    def start(queue, step, lo, hi, first=0, end=_STEPS):
        for p0, p1, units in phases:
            s0, s1 = max(p0, first), min(p1, end)
            if hi < s0 or lo >= s1 or s0 >= s1:
                continue

            def go(p0=p0, units=units):
                p = step - p0
                if units is None:
                    src, dst = pieces(("b_wo", "a_wo")[queue], 56 + (p & 7), (p >> 2) & 2)
                else:
                    turn = p >> (len(units).bit_length() - 1)
                    src, dst = pieces(units[(lo - p0) % len(units)], turn, 2 * queue)
                pltpu.make_async_copy(src, dst, sems[queue].at[step & (_RING - 1)]).start(priority=queue)

            if s0 <= lo and hi < s1:
                go()
            else:
                pl.when((step >= s0) & (step < s1))(go)

    def finish(queue, step):
        same_size = b_wq.at[pl.ds(0, 2), pl.ds(0, 64)]
        pltpu.make_async_copy(same_size, same_size, sems[queue].at[step & (_RING - 1)]).wait()

    gap = _LEAD[1] - _LEAD[0]

    def refill(step, lo, hi):
        start(0, step + _LEAD[0], lo + _LEAD[0], hi + _LEAD[0], end=_STEPS - gap)
        start(1, step + _LEAD[1], lo + _LEAD[1], hi + _LEAD[1])
        start(0, step + _LATE, lo + _LATE, hi + _LATE, first=_STEPS - gap)

    now = [0]

    def run(trips, n, body=None, carry=0, needs=()):
        idle_until(max([ready[u] for u in needs], default=0))
        s0 = now[0]
        now[0] = s0 + trips * n
        assert trips == 1 or not any(
            units and n % len(units) and s0 + _LATE < p1 and now[0] + max(_LEAD) > p0
            for p0, p1, units in phases)

        def trip(t, carry):
            used = [0]

            def tick(count=1):
                for _ in range(count):
                    lo = s0 + used[0]
                    hi = lo + (trips - 1) * n
                    step = lo + t * n
                    finish(1, step)
                    finish(0, step)
                    refill(step, lo, hi)
                    used[0] += 1

            if body is not None:
                carry = body(t, tick, carry)
            assert used[0] <= n
            tick(n - used[0])
            return carry

        return trip(0, carry) if trips == 1 else lax.fori_loop(0, trips, trip, carry)

    def idle_until(step):
        if step - now[0] >= 8:
            run((step - now[0]) // 4, 4)
        if step > now[0]:
            run(1, step - now[0])

    def fill(t, carry):
        for u in range(4):
            lo = u - ahead
            refill(lo + 4 * t, lo, lo + ahead - 4)
        return carry

    ahead = -(-max(_LEAD) // 4) * 4
    lax.fori_loop(0, ahead // 4, fill, 0)
    x_copies = (pltpu.make_async_copy(a_x_hbm, a_x, x_sems.at[0]),
                pltpu.make_async_copy(b_x_hbm, b_x, x_sems.at[1]))
    for copy in x_copies:
        copy.start()
    idle_until(16)
    for copy in x_copies:
        copy.wait()

    scale = D ** -0.5
    row8 = _iota((8, D), 0)

    def x_column(t, tick, carry):
        xrow = b_x[...].astype(_F32)
        for g in range(M // D):
            tick()
            xcol_s[g * D:(g + 1) * D, :] = jnp.broadcast_to(xrow[:, g * D:(g + 1) * D], (D, D)).T
            tick(2)
        return carry

    run(1, 12, x_column)

    def b_query(t, tick, acc):
        for part in range(4):
            tick()
            x = xcol_s.at[_ds((t * 4 + part) * 32, 32)]
            for u in range(32):
                row = (part * 32 + u) * H
                acc = acc + b_wq[t, row:row + H, :].astype(_F32) * x[u:u + 1, :]
        return acc

    qb = run(4, 4, b_query, jnp.zeros((H, D), _F32), ("b_wq",)).astype(_BF)

    own_head = (_iota((H, D), 1) & (H - 1)) == _iota((H, D), 0)

    def b_absorb(t, tick, carry):
        for half in range(2):
            tick()
            for u in (2 * half, 2 * half + 1):
                r = _dot(qb, uk[t, u * 1024:(u + 1) * 1024, :], _NT)
                z = jnp.zeros((8, D), _F32)
                for j in range(8):
                    diag = jnp.sum(jnp.where(own_head, r[:, j * D:(j + 1) * D], 0.0), axis=0, keepdims=True)
                    z = jnp.where(row8 == j, diag, z)
                z_s[_ds(t * 32 + u * 8, 8), :] = z
            tick(4)
        return carry

    run(4, 10, b_absorb, 0, ("b_uk",))

    def b_reorder(t, tick, carry):
        tick()
        zt = z_s[...].T.astype(_BF)
        lhs = jnp.concatenate([zt[j * H:(j + 1) * H, :] for j in range(4)], axis=1)
        tick()
        src = _iota((DC, DC), 0)
        order = (_iota((DC, DC), 1) == 4 * (src & (D - 1)) + (src >> 7)).astype(_BF)
        tick()
        return _dot(lhs, order).astype(_BF)

    q_abs = run(1, 6, b_reorder)

    def b_scores(t, tick, top):
        for half in range(2):
            tick()
            for u in (2 * half, 2 * half + 1):
                s = _dot(q_abs, c_buf[t, u * 256:(u + 1) * 256, :], _NT) * scale
                sb_s[t * 4 + u] = s
                top = jnp.maximum(top, jnp.maximum(s[:, :D], s[:, D:]))
            tick(3)
        return top

    top = run(4, 8, b_scores, jnp.full((H, D), -jnp.inf, _F32), ("b_c",))
    top = jnp.max(top, axis=1, keepdims=True)

    def b_values(t, tick, carry):
        total, acc = carry
        for half in range(2):
            tick()
            for u in (2 * half, 2 * half + 1):
                p = jnp.exp(sb_s[t * 4 + u] - top)
                total = total + p[:, :D] + p[:, D:]
                acc = acc + _dot(p.astype(_BF), c_buf[t, u * 256:(u + 1) * 256, :])
            tick(3)
        return total, acc

    total, lat = run(4, 8, b_values, (jnp.zeros((H, D), _F32), jnp.zeros((H, DC), _F32)))
    lat = lat / jnp.sum(total, axis=1, keepdims=True)
    lat = pltpu.bitcast(lat.astype(_BF), jnp.uint32)
    lat = jnp.concatenate([lat[:, g * D:(g + 1) * D] for g in range(DC // D)], axis=0)

    lane = _iota(lat.shape, 1)
    low_head = 2 * (_iota(lat.shape, 0) & (H // 2 - 1))
    keep = jnp.where((lane & (H - 1)) == low_head, np.uint32(0x0000FFFF),
                     jnp.where((lane & (H - 1)) == low_head + 1, np.uint32(0xFFFF0000), np.uint32(0)))

    def b_spread(t, tick, carry):
        for j in range(8):
            if j < 6:
                tick()
            words = jnp.take_along_axis(lat, (lane >> 5) + 32 * t + 4 * j, axis=1) & keep
            for g in range(DC // D):
                part = words[g * (H // 2):(g + 1) * (H // 2), :]
                latx_s[g * 4 + t, :, j * D:(j + 1) * D] = pltpu.bitcast(part, _BF)
        return carry

    run(4, 6, b_spread)

    def b_context(t, tick, acc):
        for half in range(2):
            tick()
            for u in (2 * half, 2 * half + 1):
                acc = acc + _dot(latx_s[t * 4 + u], uv[t, u * 1024:(u + 1) * 1024, :])
            tick(2)
        return acc

    ctx_s[...] = run(4, 6, b_context, jnp.zeros((H, D), _F32), ("b_uv",))

    x8 = jnp.broadcast_to(a_x[...].astype(_F32), (8, M)).astype(_BF)

    def a_query(g, tick, carry):
        q = jnp.zeros((8, D), _F32)
        for half in range(2):
            tick()
            r = _dot(x8, a_wq[:, :, _ds((g * 2 + half) * 4 * D, 4 * D)].reshape(M, 4 * D))
            for u in range(4):
                q = jnp.where(row8 == 4 * half + u, r[:, u * D:(u + 1) * D], q)
            tick(2)
        q_s[g] = q
        return carry

    run(4, 6, a_query, 0, ("a_wq",))

    row8w = _iota((8, W), 0)

    def a_scores(t, tick, s):
        q = q_s[t >> 1].astype(_BF)
        for half in range(2):
            tick()
            for u in (2 * half, 2 * half + 1):
                s = jnp.where(row8w == (t & 1) * 4 + u, _dot(q, k_buf[t * 4 + u], _NT), s)
            tick(3)
        sa_s[t >> 1] = s
        return s

    run(8, 8, a_scores, jnp.zeros((8, W), _F32), ("k0", "k1"))

    def a_softmax(t, tick, carry):
        for g in (2 * t, 2 * t + 1):
            tick()
            top = jnp.max(sa_s[g] * scale, axis=1, keepdims=True)
            tick()
            p = jnp.exp(sa_s[g] * scale - top)
            pa_s[g] = p.astype(_BF)
            l_s[_ds(g * 8, 8), :] = jnp.broadcast_to(jnp.sum(p, axis=1, keepdims=True), (8, D))
            tick()
        return carry

    run(2, 6, a_softmax)

    def a_values(g, tick, carry):
        o = jnp.zeros((8, D), _F32)
        for pair in range(4):
            tick()
            for u in (2 * pair, 2 * pair + 1):
                o = jnp.where(row8 == u, _dot(pa_s[g], v_buf[g * 8 + u]), o)
            tick(2)
        o_s[_ds(g * 8, 8), :] = o
        return carry

    run(2, 12, a_values, 0, ("v0",))
    run(2, 12, lambda g, tick, carry: a_values(g + 2, tick, carry), 0, ("v1",))
    o_s[...] = o_s[...] / l_s[...]

    def flatten(t, tick, carry):
        for r in (2 * t, 2 * t + 1):
            tick()
            for branch, src in enumerate((ctx_s, o_s)):
                rows = [jnp.broadcast_to(src[pl.ds(8 * q + r, 1), :], (8, D)) for q in range(4)]
                flat_s[branch, r] = jnp.concatenate(rows, axis=1).astype(_BF)
        return carry

    run(4, 2, flatten)

    def column(t, tick, carry):
        for branch, src in enumerate((ctx_s, o_s)):
            tick()
            row = src[pl.ds(8 * (2 + t) + 7, 1), :].astype(_BF).astype(_F32)
            ocol_s[branch, t] = jnp.broadcast_to(row, (D, D)).T
            tick(2)
        return carry

    run(2, 6, column)

    def project(acc, branch, r, q0, nq):
        w = (b_wo, a_wo)[branch][pl.ds(q0, nq), _ds(r * D, D), :].reshape(nq * D, M)
        return acc + _dot(flat_s[branch, r, :, _ds(q0 * D, nq * D)], w)

    def rounds_from(r0):
        def body(t, tick, acc):
            acc = list(acc)
            for branch in range(2):
                tick()
                acc[branch] = project(acc[branch], branch, r0 + t, 0, 4)
                tick(2)
            return tuple(acc)
        return body

    acc = (jnp.zeros((8, M), _F32), jnp.zeros((8, M), _F32))
    r = 0
    while r < 7:
        idle_until(_PROJ + 16 * (r + 1))
        landed = min(7, (now[0] - _PROJ) // 16)
        acc = run(landed - r, 6, rounds_from(r), acc)
        r = landed
    idle_until(_HALF + 8)
    acc = [project(acc[branch], branch, 7, 0, 2) for branch in range(2)]

    part = [jnp.where(_iota((8, M), 0) == 0, x, 0.0) for x in acc]
    last, p = now[0], 0
    assert last == _STEPS - 8
    for count in _GROUPS:
        r0, n = 16 * p, 16 * count
        for step in range(last + p, last + p + count):
            finish(0, step)
            finish(1, step)
            refill(step, step, step)
        for branch, w_ref in enumerate((b_wo, a_wo)):
            for q in range(2):
                w = w_ref[2 + q, 7 * D + r0:7 * D + r0 + n, :].astype(_F32)
                prod = w * jnp.concatenate([ocol_s[branch, q, r0:r0 + n, :]] * (M // D), axis=1)
                rows = [prod[8 * j:8 * j + 8] for j in range(n // 8)]
                while len(rows) > 1:
                    rows = [rows[j] + rows[j + 1] for j in range(0, len(rows), 2)]
                part[branch] = part[branch] + rows[0]
        p += count
    assert last + p == _STEPS
    out = jnp.concatenate([jnp.sum(x, axis=0, keepdims=True) for x in part[::-1]], axis=1)
    out_ref[...] = out.astype(out_ref.dtype)


@jax.jit
def pallas_concat_heads__sliding_block_cached__compressed_kv_cla__decode_kernel(
        A_x, A_k_cache, A_v_cache, A_wq, A_wo, B_x, B_c_kv, B_w_q, B_w_uk, B_w_uv, B_w_o):
    assert A_k_cache.shape == A_v_cache.shape == (1, H, SK, D) and B_c_kv.shape == (1, SK, DC)
    assert B_w_q.shape == (M, H, D) and B_w_uk.shape == B_w_uv.shape == (DC, H, D)
    operands = (
        A_x.reshape(1, M), A_k_cache.reshape(H, SK, D), A_v_cache.reshape(H, SK, D),
        A_wq.reshape(4, M // 4, H * D), A_wo.reshape(4, H * D // 4, M),
        B_x.reshape(1, M), B_c_kv.reshape(4, SK // 4, DC), B_w_q.reshape(4, M * H // 4, D),
        B_w_uk.reshape(4, DC * H // 4, D), B_w_uv.reshape(4, DC * H // 4, D),
        B_w_o.reshape(4, H * D // 4, M))
    buffers = [pltpu.VMEM((H, W, D) if i in (1, 2) else x.shape, _BF) for i, x in enumerate(operands)]
    out = pl.pallas_call(
        _kernel,
        in_specs=[pl.BlockSpec(memory_space=pltpu.HBM)] * len(operands),
        out_specs=pl.BlockSpec(memory_space=pltpu.VMEM),
        out_shape=jax.ShapeDtypeStruct((1, 2 * M), A_x.dtype),
        scratch_shapes=buffers + [
            pltpu.VMEM((M, D), _F32),
            pltpu.VMEM((D, D), _F32),
            pltpu.VMEM((SK // 256, H, 256), _F32),
            pltpu.VMEM((DC * H // 1024, H, 1024), _BF),
            pltpu.VMEM((H, D), _F32),
            pltpu.VMEM((H // 8, 8, D), _F32),
            pltpu.VMEM((H // 8, 8, W), _F32),
            pltpu.VMEM((H // 8, 8, W), _BF),
            pltpu.VMEM((H, D), _F32),
            pltpu.VMEM((H, D), _F32),
            pltpu.VMEM((2, 8, 8, 4 * D), _BF),
            pltpu.VMEM((2, 2, D, D), _F32),
            pltpu.SemaphoreType.DMA((_RING,)),
            pltpu.SemaphoreType.DMA((_RING,)),
            pltpu.SemaphoreType.DMA((2,)),
        ],
        compiler_params=pltpu.CompilerParams(
            vmem_limit_bytes=64 * 1024 * 1024,
            disable_bounds_checks=True,
            disable_semaphore_checks=True),
    )(*operands)
    return out.reshape(1, 1, 2 * M)
```

```python
import jax
import jax.numpy as jnp
import numpy as np
from jax import lax
import jax.experimental.pallas as pl
import jax.experimental.pallas.tpu as pltpu

H = 32
D = 128
M = 512
DC = 512
SK = 4096
W = min(4096, max(256, SK // 4))

_BF = jnp.bfloat16
_F32 = jnp.float32
_NN = (((1,), (0,)), ((), ()))
_NT = (((1,), (1,)), ((), ()))

_ORDER = (("b_c", "b_wq", "b_uk", "b_uv"), ("k0", "a_wq"), ("k1",), ("v0",), ("v1",))
_PROJ = 576
_HALF = 688
_STEPS = 704
_LEAD = (30, 56)
_LATE = 12
_GROUPS = (4, 2, 1, 1)
_RING = 64


def _phases():
    phases, ready, s = [], {}, 0
    for units in _ORDER:
        phases.append((s, s + 64 * len(units), units))
        s += 64 * len(units)
        ready.update({u: s for u in units})
    assert s == _PROJ
    phases += [(_PROJ, _HALF, ("b_wo", "a_wo")), (_HALF, _STEPS, None)]
    return phases, ready


def _dot(a, b, dims=_NN):
    return lax.dot_general(a, b, dims, preferred_element_type=_F32)


def _iota(shape, dim):
    return lax.broadcasted_iota(jnp.int32, shape, dim)


def _ds(start, size):
    return pl.ds(start if isinstance(start, int) else pl.multiple_of(start, size), size)


def _kernel(a_x_hbm, k_hbm, v_hbm, a_wq_hbm, a_wo_hbm,
            b_x_hbm, c_hbm, b_wq_hbm, uk_hbm, uv_hbm, b_wo_hbm,
            out_ref,
            a_x, k_buf, v_buf, a_wq, a_wo, b_x, c_buf, b_wq, uk, uv, b_wo,
            xcol_s, z_s, sb_s, latx_s, ctx_s, q_s, sa_s, pa_s, l_s, o_s, flat_s, ocol_s,
            sem0, sem1, x_sems):
    phases, ready = _phases()
    sems = (sem0, sem1)
    weights = dict(b_wq=(b_wq_hbm, b_wq), b_uk=(uk_hbm, uk), b_uv=(uv_hbm, uv), b_c=(c_hbm, c_buf),
                   a_wq=(a_wq_hbm, a_wq), b_wo=(b_wo_hbm, b_wo), a_wo=(a_wo_hbm, a_wo))

    def pieces(unit, i, first):
        if unit[0] in "kv":
            src, dst = (k_hbm, k_buf) if unit[0] == "k" else (v_hbm, v_buf)
            heads = pl.ds(int(unit[1]) * 16 + (i & 3) * 4 + first, 2)
            row = (i >> 2) * 64
            return src.at[heads, _ds(SK - W + row, 64)], dst.at[heads, _ds(row, 64)]
        if unit == "a_wq":
            idx = (pl.ds(first, 2), _ds((i >> 2) * 8, 8), _ds((i & 3) * 1024, 1024))
        elif unit in ("b_wq", "b_uk", "b_uv"):
            idx = (pl.ds(first, 2), _ds(i * 64, 64))
        else:
            idx = (pl.ds(first, 2), _ds(i * 16, 16))
        src, dst = weights[unit]
        return src.at[idx], dst.at[idx]

    def with_copy(act, queue, step, lo, hi, first=0, end=_STEPS):
        for p0, p1, units in phases:
            s0, s1 = max(p0, first), min(p1, end)
            if hi < s0 or lo >= s1 or s0 >= s1:
                continue

            def go(p0=p0, units=units):
                p = step - p0
                if units is None:
                    src, dst = pieces(("b_wo", "a_wo")[queue], 56 + (p & 7), (p >> 2) & 2)
                else:
                    turn = p >> (len(units).bit_length() - 1)
                    src, dst = pieces(units[(lo - p0) % len(units)], turn, 2 * queue)
                act(pltpu.make_async_copy(src, dst, sems[queue].at[step & (_RING - 1)]))

            if s0 <= lo and hi < s1:
                go()
            else:
                pl.when((step >= s0) & (step < s1))(go)

    def start(queue, *args, **kwargs):
        with_copy(lambda copy: copy.start(priority=queue), queue, *args, **kwargs)

    def finish(queue, step, lo, hi):
        with_copy(lambda copy: copy.wait(), queue, step, lo, hi)

    gap = _LEAD[1] - _LEAD[0]

    def refill(step, lo, hi):
        start(0, step + _LEAD[0], lo + _LEAD[0], hi + _LEAD[0], end=_STEPS - gap)
        start(1, step + _LEAD[1], lo + _LEAD[1], hi + _LEAD[1], first=1)
        start(0, step + _LATE, lo + _LATE, hi + _LATE, first=_STEPS - gap)

    now = [0]

    def run(trips, n, body=None, carry=0, needs=()):
        idle_until(max([ready[u] for u in needs], default=0))
        s0 = now[0]
        now[0] = s0 + trips * n
        assert trips == 1 or not any(
            units and n % len(units) and s0 < p1 and now[0] + max(_LEAD) > p0
            for p0, p1, units in phases)

        def trip(t, carry):
            used = [0]

            def tick(count=1):
                for _ in range(count):
                    lo = s0 + used[0]
                    hi = lo + (trips - 1) * n
                    step = lo + t * n
                    finish(1, step, lo, hi)
                    finish(0, step, lo, hi)
                    refill(step, lo, hi)
                    used[0] += 1

            if body is not None:
                carry = body(t, tick, carry)
            assert used[0] <= n
            tick(n - used[0])
            return carry

        return trip(0, carry) if trips == 1 else lax.fori_loop(0, trips, trip, carry)

    def idle_until(step):
        if step - now[0] >= 8:
            run((step - now[0]) // 4, 4)
        if step > now[0]:
            run(1, step - now[0])

    def fill(t, carry):
        for u in range(4):
            lo = u - ahead
            refill(lo + 4 * t, lo, lo + ahead - 4)
        return carry

    start(1, 0, 0, 0)
    ahead = -(-max(_LEAD) // 4) * 4
    lax.fori_loop(0, ahead // 4, fill, 0)
    x_copies = (pltpu.make_async_copy(a_x_hbm, a_x, x_sems.at[0]),
                pltpu.make_async_copy(b_x_hbm, b_x, x_sems.at[1]))
    for copy in x_copies:
        copy.start()
    idle_until(16)
    for copy in x_copies:
        copy.wait()

    scale = D ** -0.5
    row8 = _iota((8, D), 0)

    def x_column(t, tick, carry):
        xrow = b_x[...].astype(_F32)
        for g in range(M // D):
            tick()
            xcol_s[g * D:(g + 1) * D, :] = jnp.broadcast_to(xrow[:, g * D:(g + 1) * D], (D, D)).T
            tick(2)
        return carry

    run(1, 12, x_column)

    def b_query(t, tick, acc):
        for part in range(4):
            tick()
            x = xcol_s.at[_ds((t * 4 + part) * 32, 32)]
            for u in range(32):
                row = (part * 32 + u) * H
                acc = acc + b_wq[t, row:row + H, :].astype(_F32) * x[u:u + 1, :]
        return acc

    qb = run(4, 4, b_query, jnp.zeros((H, D), _F32), ("b_wq",)).astype(_BF)

    own_head = (_iota((H, D), 1) & (H - 1)) == _iota((H, D), 0)

    def b_absorb(t, tick, carry):
        for half in range(2):
            tick()
            for u in (2 * half, 2 * half + 1):
                r = _dot(qb, uk[t, u * 1024:(u + 1) * 1024, :], _NT)
                z = jnp.zeros((8, D), _F32)
                for j in range(8):
                    diag = jnp.sum(jnp.where(own_head, r[:, j * D:(j + 1) * D], 0.0), axis=0, keepdims=True)
                    z = jnp.where(row8 == j, diag, z)
                z_s[_ds(t * 32 + u * 8, 8), :] = z
            tick(4)
        return carry

    run(4, 10, b_absorb, 0, ("b_uk",))

    def b_reorder(t, tick, carry):
        tick()
        zt = z_s[...].T.astype(_BF)
        lhs = jnp.concatenate([zt[j * H:(j + 1) * H, :] for j in range(4)], axis=1)
        tick()
        src = _iota((DC, DC), 0)
        order = (_iota((DC, DC), 1) == 4 * (src & (D - 1)) + (src >> 7)).astype(_BF)
        tick()
        return _dot(lhs, order).astype(_BF)

    q_abs = run(1, 6, b_reorder)

    def b_scores(t, tick, top):
        for half in range(2):
            tick()
            for u in (2 * half, 2 * half + 1):
                s = _dot(q_abs, c_buf[t, u * 256:(u + 1) * 256, :], _NT) * scale
                sb_s[t * 4 + u] = s
                top = jnp.maximum(top, jnp.maximum(s[:, :D], s[:, D:]))
            tick(3)
        return top

    top = run(4, 8, b_scores, jnp.full((H, D), -jnp.inf, _F32), ("b_c",))
    top = jnp.max(top, axis=1, keepdims=True)

    def b_values(t, tick, carry):
        total, acc = carry
        for half in range(2):
            tick()
            for u in (2 * half, 2 * half + 1):
                p = jnp.exp(sb_s[t * 4 + u] - top)
                total = total + p[:, :D] + p[:, D:]
                acc = acc + _dot(p.astype(_BF), c_buf[t, u * 256:(u + 1) * 256, :])
            tick(3)
        return total, acc

    total, lat = run(4, 8, b_values, (jnp.zeros((H, D), _F32), jnp.zeros((H, DC), _F32)))
    lat = lat / jnp.sum(total, axis=1, keepdims=True)
    lat = pltpu.bitcast(lat.astype(_BF), jnp.uint32)
    lat = jnp.concatenate([lat[:, g * D:(g + 1) * D] for g in range(DC // D)], axis=0)

    lane = _iota(lat.shape, 1)
    low_head = 2 * (_iota(lat.shape, 0) & (H // 2 - 1))
    keep = jnp.where((lane & (H - 1)) == low_head, np.uint32(0x0000FFFF),
                     jnp.where((lane & (H - 1)) == low_head + 1, np.uint32(0xFFFF0000), np.uint32(0)))

    def b_spread(t, tick, carry):
        for j in range(8):
            if j < 6:
                tick()
            words = jnp.take_along_axis(lat, (lane >> 5) + 32 * t + 4 * j, axis=1) & keep
            for g in range(DC // D):
                part = words[g * (H // 2):(g + 1) * (H // 2), :]
                latx_s[g * 4 + t, :, j * D:(j + 1) * D] = pltpu.bitcast(part, _BF)
        return carry

    run(4, 6, b_spread)

    def b_context(t, tick, acc):
        for half in range(2):
            tick()
            for u in (2 * half, 2 * half + 1):
                acc = acc + _dot(latx_s[t * 4 + u], uv[t, u * 1024:(u + 1) * 1024, :])
            tick(2)
        return acc

    ctx_s[...] = run(4, 6, b_context, jnp.zeros((H, D), _F32), ("b_uv",))

    x8 = jnp.broadcast_to(a_x[...].astype(_F32), (8, M)).astype(_BF)

    def a_query(g, tick, carry):
        q = jnp.zeros((8, D), _F32)
        for half in range(2):
            tick()
            r = _dot(x8, a_wq[:, :, _ds((g * 2 + half) * 4 * D, 4 * D)].reshape(M, 4 * D))
            for u in range(4):
                q = jnp.where(row8 == 4 * half + u, r[:, u * D:(u + 1) * D], q)
            tick(2)
        q_s[g] = q
        return carry

    run(4, 6, a_query, 0, ("a_wq",))

    row8w = _iota((8, W), 0)

    def a_scores(t, tick, s):
        q = q_s[t >> 1].astype(_BF)
        for half in range(2):
            tick()
            for u in (2 * half, 2 * half + 1):
                s = jnp.where(row8w == (t & 1) * 4 + u, _dot(q, k_buf[t * 4 + u], _NT), s)
            tick(3)
        sa_s[t >> 1] = s
        return s

    run(8, 8, a_scores, jnp.zeros((8, W), _F32), ("k0", "k1"))

    def a_softmax(t, tick, carry):
        for g in (2 * t, 2 * t + 1):
            tick()
            top = jnp.max(sa_s[g] * scale, axis=1, keepdims=True)
            tick()
            p = jnp.exp(sa_s[g] * scale - top)
            pa_s[g] = p.astype(_BF)
            l_s[_ds(g * 8, 8), :] = jnp.broadcast_to(jnp.sum(p, axis=1, keepdims=True), (8, D))
            tick()
        return carry

    run(2, 6, a_softmax)

    def a_values(g, tick, carry):
        o = jnp.zeros((8, D), _F32)
        for pair in range(4):
            tick()
            for u in (2 * pair, 2 * pair + 1):
                o = jnp.where(row8 == u, _dot(pa_s[g], v_buf[g * 8 + u]), o)
            tick(2)
        o_s[_ds(g * 8, 8), :] = o
        return carry

    run(2, 12, a_values, 0, ("v0",))
    run(2, 12, lambda g, tick, carry: a_values(g + 2, tick, carry), 0, ("v1",))
    o_s[...] = o_s[...] / l_s[...]

    def flatten(t, tick, carry):
        for r in (2 * t, 2 * t + 1):
            tick()
            for branch, src in enumerate((ctx_s, o_s)):
                rows = [jnp.broadcast_to(src[pl.ds(8 * q + r, 1), :], (8, D)) for q in range(4)]
                flat_s[branch, r] = jnp.concatenate(rows, axis=1).astype(_BF)
        return carry

    run(4, 2, flatten)

    def column(t, tick, carry):
        for branch, src in enumerate((ctx_s, o_s)):
            tick()
            row = src[pl.ds(8 * (2 + t) + 7, 1), :].astype(_BF).astype(_F32)
            ocol_s[branch, t] = jnp.broadcast_to(row, (D, D)).T
            tick(2)
        return carry

    run(2, 6, column)

    def project(acc, branch, r, q0, nq):
        w = (b_wo, a_wo)[branch][pl.ds(q0, nq), _ds(r * D, D), :].reshape(nq * D, M)
        return acc + _dot(flat_s[branch, r, :, _ds(q0 * D, nq * D)], w)

    def rounds_from(r0):
        def body(t, tick, acc):
            acc = list(acc)
            for branch in range(2):
                tick()
                acc[branch] = project(acc[branch], branch, r0 + t, 0, 4)
                tick(2)
            return tuple(acc)
        return body

    acc = (jnp.zeros((8, M), _F32), jnp.zeros((8, M), _F32))
    r = 0
    while r < 7:
        idle_until(_PROJ + 16 * (r + 1))
        landed = min(7, (now[0] - _PROJ) // 16)
        acc = run(landed - r, 6, rounds_from(r), acc)
        r = landed
    idle_until(_HALF + 8)
    acc = [project(acc[branch], branch, 7, 0, 2) for branch in range(2)]

    part = [jnp.where(_iota((8, M), 0) == 0, x, 0.0) for x in acc]
    last, p = now[0], 0
    assert last == _STEPS - 8 and last + _LATE >= _STEPS
    for count in _GROUPS:
        r0, n = 16 * p, 16 * count
        for step in range(last + p, last + p + count):
            finish(0, step, step, step)
            finish(1, step, step, step)
        for branch, w_ref in enumerate((b_wo, a_wo)):
            for q in range(2):
                w = w_ref[2 + q, 7 * D + r0:7 * D + r0 + n, :].astype(_F32)
                prod = w * jnp.concatenate([ocol_s[branch, q, r0:r0 + n, :]] * (M // D), axis=1)
                rows = [prod[8 * j:8 * j + 8] for j in range(n // 8)]
                while len(rows) > 1:
                    rows = [rows[j] + rows[j + 1] for j in range(0, len(rows), 2)]
                part[branch] = part[branch] + rows[0]
        p += count
    assert last + p == _STEPS
    out_ref[:, M:] = jnp.sum(part[0], axis=0, keepdims=True).astype(out_ref.dtype)
    out_ref[:, :M] = jnp.sum(part[1], axis=0, keepdims=True).astype(out_ref.dtype)


@jax.jit
def pallas_concat_heads__sliding_block_cached__compressed_kv_cla__decode_kernel(
        A_x, A_k_cache, A_v_cache, A_wq, A_wo, B_x, B_c_kv, B_w_q, B_w_uk, B_w_uv, B_w_o):
    assert A_k_cache.shape == A_v_cache.shape == (1, H, SK, D) and B_c_kv.shape == (1, SK, DC)
    assert B_w_q.shape == (M, H, D) and B_w_uk.shape == B_w_uv.shape == (DC, H, D)
    operands = (
        A_x.reshape(1, M), A_k_cache.reshape(H, SK, D), A_v_cache.reshape(H, SK, D),
        A_wq.reshape(4, M // 4, H * D), A_wo.reshape(4, H * D // 4, M),
        B_x.reshape(1, M), B_c_kv.reshape(4, SK // 4, DC), B_w_q.reshape(4, M * H // 4, D),
        B_w_uk.reshape(4, DC * H // 4, D), B_w_uv.reshape(4, DC * H // 4, D),
        B_w_o.reshape(4, H * D // 4, M))
    buffers = [pltpu.VMEM((H, W, D) if i in (1, 2) else x.shape, _BF) for i, x in enumerate(operands)]
    out = pl.pallas_call(
        _kernel,
        in_specs=[pl.BlockSpec(memory_space=pltpu.HBM)] * len(operands),
        out_specs=pl.BlockSpec(memory_space=pltpu.VMEM),
        out_shape=jax.ShapeDtypeStruct((1, 2 * M), A_x.dtype),
        scratch_shapes=buffers + [
            pltpu.VMEM((M, D), _F32),
            pltpu.VMEM((D, D), _F32),
            pltpu.VMEM((SK // 256, H, 256), _F32),
            pltpu.VMEM((DC * H // 1024, H, 1024), _BF),
            pltpu.VMEM((H, D), _F32),
            pltpu.VMEM((H // 8, 8, D), _F32),
            pltpu.VMEM((H // 8, 8, W), _F32),
            pltpu.VMEM((H // 8, 8, W), _BF),
            pltpu.VMEM((H, D), _F32),
            pltpu.VMEM((H, D), _F32),
            pltpu.VMEM((2, 8, 8, 4 * D), _BF),
            pltpu.VMEM((2, 2, D, D), _F32),
            pltpu.SemaphoreType.DMA((_RING,)),
            pltpu.SemaphoreType.DMA((_RING,)),
            pltpu.SemaphoreType.DMA((2,)),
        ],
        compiler_params=pltpu.CompilerParams(
            vmem_limit_bytes=64 * 1024 * 1024,
            disable_bounds_checks=True,
            disable_semaphore_checks=True),
    )(*operands)
    return out.reshape(1, 1, 2 * M)
```
